```python
import os as _os
_os.environ.setdefault("JAX_PLATFORMS", "cpu")
import jax
import jax.numpy as jnp

def _softmax(x, axis=-1):
    return jax.nn.softmax(x, axis=axis)
def _gelu(x):
    return jax.nn.gelu(x, approximate=True)
def _silu(x):
    return jax.nn.silu(x)
def _sigmoid(x):
    return jax.nn.sigmoid(x)
def _layernorm(x, axis=-1, eps=1e-5):
    m = jnp.mean(x, axis=axis, keepdims=True)
    v = jnp.var(x, axis=axis, keepdims=True)
    return (x - m) / jnp.sqrt(v + eps)
def _scatter_add(tgt, idx, src, axis=0):
    return tgt.at[idx].add(src)
def _segment_sum(src, seg, n):
    return jax.ops.segment_sum(src, seg, n)
class _Rng:
    def __init__(self, key):
        self._k = key
    def _next(self):
        self._k, sub = jax.random.split(self._k)
        return sub
    def normal(self, shape):
        return jax.random.normal(self._next(), shape, dtype=jnp.bfloat16)
    def randint(self, lo, hi, shape):
        return jax.random.randint(self._next(), shape, lo, hi, dtype=jnp.int32)
    def uniform(self, shape, lo=0.0, hi=1.0):
        return jax.random.uniform(self._next(), shape, jnp.bfloat16, lo, hi)
    def permutation(self, n):
        return jax.random.permutation(self._next(), n)


kernel_name = 'interleave_layers__ssm_conv_h3__mixer_s_mlp__prompt'

def setup_inputs():
    _rng = _Rng(jax.random.key(int.from_bytes(__import__("os").urandom(4), "little")))
    _w = (lambda a: (lambda t: t.astype(jnp.bfloat16) if jnp.issubdtype(t.dtype, jnp.floating) else t)(jnp.asarray(a)))
    def _A_setup():
        B, S, D = 1, 2048, 640
        ks = 4
        return {
            "q": _w((lambda *s: _rng.normal(s) * 0.05)(B, S, D)),
            "k": _w((lambda *s: _rng.normal(s) * 0.4)(B, S, D)),
            "v": _w((lambda *s: _rng.normal(s) * 0.4)(B, S, D)),
            "shift_k": _w((lambda *s: _rng.normal(s) * 0.4)(D, ks) * 0.5),
            "ssm_k": _w((lambda *s: _rng.normal(s) * 0.4)(D, S) * (1.0 / S ** 0.5)),
            "ssm_D": _w((lambda *s: _rng.normal(s) * 0.4)(D)),
        }
    _A_in = _A_setup()

    def _B_setup():
        B, S, D, F = 1, 2048, 640, 1536
        return {
            "x":  _w((lambda *s: _rng.normal(s) * 0.05)(B, S, D)),
            "w1": _w((lambda *s: _rng.normal(s) * 0.8)(D, D) * (D ** -0.5)),
            "w2": _w((lambda *s: _rng.normal(s) * 0.8)(D, D) * (D ** -0.5)),
            "w3": _w((lambda *s: _rng.normal(s) * 0.8)(D, F) * (D ** -0.5)),
            "w4": _w((lambda *s: _rng.normal(s) * 0.8)(F, D) * (F ** -0.5)),
        }
    _B_in = _B_setup()

    return {
        "A_q": _A_in["q"],
        "A_k": _A_in["k"],
        "A_v": _A_in["v"],
        "A_shift_k": _A_in["shift_k"],
        "A_ssm_k": _A_in["ssm_k"],
        "A_ssm_D": _A_in["ssm_D"],
        "B_x": _B_in["x"],
        "B_w1": _B_in["w1"],
        "B_w2": _B_in["w2"],
        "B_w3": _B_in["w3"],
        "B_w4": _B_in["w4"],
    }

def reference(A_q, A_k, A_v, A_shift_k, A_ssm_k, A_ssm_D, B_x, B_w1, B_w2, B_w3, B_w4):
    def _A_ref(q, k, v, shift_k, ssm_k, ssm_D):
        B, S, D = q.shape
        ks = shift_k.shape[-1]
        k_pad = jnp.pad(k, ((0, 0), (ks - 1, 0), (0, 0)))
        k_shift = jnp.zeros_like(k)
        for t in range(ks):
            k_shift = k_shift + k_pad[:, t:t + S, :] * shift_k[:, ks - 1 - t][None, None, :]
        kv = k_shift * v
        L = 2 * S
        kv_pad = jnp.pad(kv, ((0, 0), (0, S), (0, 0)))
        kf_pad = jnp.pad(ssm_k, ((0, 0), (0, S)))
        kv_f = (lambda x, axes=(-2,-1): jnp.fft.rfft2(x.astype(jnp.float32), axes=axes))(kv_pad[:, None, :, :], axes=(1, 2))
        kf_f = (lambda x, axes=(-2,-1): jnp.fft.rfft2(x.astype(jnp.float32), axes=axes))(kf_pad[:, None, :], axes=(1, 2))
        kf_f = (lambda x, *d: x.transpose(*d))(kf_f, 1, 2, 0)
        y_f = kv_f * kf_f[None, :, :, :]
        y = (lambda x, s, axes=(-2,-1): jnp.fft.irfft2(x, s=s, axes=axes).astype(jnp.bfloat16))(y_f, (1, L), axes=(1, 2))[:, 0, :S, :]
        y = y + kv * ssm_D[None, None, :]
        return q * y

    def _B_ref(x, w1, w2, w3, w4):
        B, S, D = x.shape
        h = _gelu(_layernorm(x, axis=-1) @ w1)
        c = D // 4
        g0 = jnp.pad(h[:, :, 0*c:1*c], ((0, 0), (1, 0), (0, 0)))[:, :S, :]
        g1 = jnp.pad(h[:, :, 1*c:2*c], ((0, 0), (0, 1), (0, 0)))[:, 1:, :]
        g2 = jnp.pad(h[:, :, 2*c:3*c], ((0, 0), (2, 0), (0, 0)))[:, :S, :]
        g3 = jnp.pad(h[:, :, 3*c:   ], ((0, 0), (0, 2), (0, 0)))[:, 2:, :]
        hs = jnp.concatenate([g0, g1, g2, g3], axis=-1) @ w2
        x1 = x + hs
        h2 = _gelu(_layernorm(x1, axis=-1) @ w3) @ w4
        return x1 + h2

    x = A_q
    x = x + _A_ref(_layernorm(x, axis=-1), A_k, A_v, A_shift_k, A_ssm_k, A_ssm_D)
    x = x + _B_ref(_layernorm(x, axis=-1), B_w1, B_w2, B_w3, B_w4)
    x = x + _A_ref(_layernorm(x, axis=-1), A_k, A_v, A_shift_k, A_ssm_k, A_ssm_D)
    x = x + _B_ref(_layernorm(x, axis=-1), B_w1, B_w2, B_w3, B_w4)
    return x
```

```python
import numpy as np
import jax
import jax.numpy as jnp
from jax import lax
import jax.experimental.pallas as pl
import jax.experimental.pallas.tpu as pltpu

S, D, F = 2048, 640, 1536
NB = D // 128
R = 4
T = 128 * R
NT = S // T
OFF = 64
HP = 8
PC = 32
EPS = 1e-5
f32, bf16, u32 = jnp.float32, jnp.bfloat16, jnp.uint32

GC = float(np.sqrt(2 / np.pi))
GS = float((GC * 0.044715) ** (1 / 3))
GO = 0.5 / GS

LAM = (-2, -1, 0, 1, 2)
STAR = (0, 1, 0), (0, 2, 2), (0, 3, 3), (0, 4, 0), (1, 2, 1), (1, 3, 1), (1, 4, 4), (2, 3, 2), (2, 4, 4), (3, 4, 3)
ORD3 = (0, 2), (0, 4), (0, 3), (0, 5), (2, 4), (2, 5), (1, 2), (1, 4), (3, 4), (1, 3), (1, 5), (3, 5)
ORD4 = (0, 2), (0, 4), (2, 4), (1, 2), (1, 4), (0, 5), (2, 5), (1, 5), (3, 5), (0, 3), (3, 4), (1, 3)
PAIR4 = (0, 2), (6, 8), (4, 1), (11, 9), (5, 3), (10, 7)

TILES = (0, 0), (1, 0), (0, 1), (0, 2), (1, 1), (0, 3), (1, 2), (1, 3)
CONV = ('u0 g0 u1 g1 y0 u2 g2 y1 u3 g3 y2 u4 g4 y3 y4', 'u0 g0 u1 g1 u2 g2 y0 y1 y2 u3 g3 u4 g4 y3 y4',
        'u0 g0 u1 g1 u2 g2 y0 u3 g3 y1 u4 g4 y2 y3 y4', 'u0 g0 u1 g1 u2 g2 y0 u3 g3 y1 u4 g4 y2 y3 y4')
CUTS = (8, 11), (10, 13), (8, 11), (10, 13), (10, 13), (8, 11)
SPANS = (3, 0, 260 + 30, 260 + 80), (2, 0, 124 + 36, 124 + 84), (1, 9, 124, 124 + 8)
WAITS = ((-1, ((0, 0),)), (1, ((0, 1),)), (3, ((0, 2),)), (6, ((0, 3), (0, 4))), (12, ('q0',)), (14, ('w1',)),
         (28, ('w2', 'w3a')), (50, ('w3b', 'w4')), (80, ((1, 0), (1, 1), (1, 2), (1, 3), (1, 4), 'q1')),
         (140, (2, 'q2')), (249, (3, 'q3')))
BIAS = ('90520914959005990985722562202947151490042228556710009445464658447699430224032541019776534124749944444344'
        '46554169420094464103949184933902455001960566487335642111398145468433445936424026340664520001725462204035'
        '46545644027934362030580663125954330415473229034416308246437587802264035574222644564546735624944457110005'
        '13905890132049940318249803441599520490761160593999021513233304845172525863488042343397444651444642473433'
        '34355400456457498246354864494727913612564320305189133731235552492533133446103964909930156638326514155138'
        '3154508220591127211176934935200334460200569454794400425775583344426544574322434344515434744200477')


def _lo(w):
    return lax.bitcast_convert_type(w << 16, f32)


def _hi(w):
    return lax.bitcast_convert_type(w & np.uint32(0xFFFF0000), f32)


def _unpack(w):
    return pltpu.bitcast(w, bf16)


def _bfly(a, inverse):
    (r0, i0), (r1, i1), (r2, i2), (r3, i3) = a
    sr, si, dr, di = r0 + r2, i0 + i2, r0 - r2, i0 - i2
    tr, ti, er, ei = r1 + r3, i1 + i3, r1 - r3, i1 - i3
    x0, x2, xm, xp = (sr + tr, si + ti), (sr - tr, si - ti), (dr + ei, di - er), (dr - ei, di + er)
    return [x0, xp, x2, xm] if inverse else [x0, xm, x2, xp]


def _sums(x):
    s = jnp.sum(x, axis=-1, keepdims=True)
    return jnp.broadcast_to(s, (x.shape[0], 128)), jnp.sum(x * x, axis=-1, keepdims=True)


def _rstd(s, q, scale):
    v = jnp.maximum(q - s * (s * (1.0 / D)), 0.0) + D * EPS
    return jnp.exp2(jnp.log(v) * float(-0.5 / np.log(2)) + float(np.log2(scale * D ** 0.5)))


def _norm(x, s, r):
    m = s * (1.0 / D)
    return jnp.concatenate([(x[:, o:o + 128] - m) * r for o in range(0, D, 128)], axis=1)


def _gelu(x):
    return x * jnp.tanh(x * (x * x + GC / GS)) + x


def _dot(a, b):
    return jnp.dot(a.astype(bf16), b, preferred_element_type=f32)


def _axpy(y, c, x):
    if y is None:
        return x if c == 1 else c * x
    return y if c == 0 else y + x if c == 1 else y - x if c == -1 else y + c * x


def _total(terms, rows):
    out = None
    for x in terms:
        out = _axpy(out, 1, x[rows])
    return out


def _again(g):
    return any(e[2] == STAR[g][2] for e in STAR[:g])


def _star_weights(b, g):
    i, j, e = STAR[g]
    d = LAM[j] - LAM[i]
    w1, w2, dg = _axpy(None, d, b[i][j]), _axpy(None, -d, b[j][i]), b[e][e]
    for o in range(NB):
        if o != e:
            dg = dg - b[e][o] if _again(g) else dg + b[o][e]
    return w1, w2, w1 - w2, dg


def _star(od, src, w):
    f, z, r = {}, [[] for _ in range(NB)], [[] for _ in range(NB)]

    def fn(i):
        if i not in f:
            a, b = src(i)
            f[i] = (a, _axpy(b, LAM[i], a))
        return f[i]

    def group(g):
        i, j, e = STAR[g]
        d = LAM[j] - LAM[i]
        (ai, pi), (aj, pj) = fn(i), fn(j)
        l3 = od.group(_axpy(None, 1 / d, pi - pj))
        p1, p2, p3, pd = (_dot(x, w(4 * g + k)) for k, x in enumerate((l3 + ai, l3 + aj, l3, fn(e)[not _again(g)])))
        od.issued(p1)
        q = _axpy(None, 1 / d, p1 - p2 - p3)
        r[j].append(p1 + pd if e == j and not _again(g) else p1)
        r[i].append(p2 + pd if e == i and not _again(g) else p2)
        z[i].append(q + pd if e == i and _again(g) else q)
        z[j].append(q + pd if e == j and _again(g) else q)

    def result(o, rows):
        assert len(z[o]) == NB - 1
        top = _total(z[o], rows)
        return top, _axpy(_total(r[o], rows), -LAM[o], top)

    return [lambda g=g: group(g) for g in range(len(STAR))], result


def _octa_weights(b, i, j):
    e, x = (j, i // 2) if (i + j) % 2 else (i, j // 2)
    dg = b(e, e)
    for o in range(6):
        if o // 2 == x:
            dg = dg + b(o, e)
        elif o // 2 != e // 2:
            dg = dg - b(e, o)
    return b(i, j), b(j, i), b(i, j) + b(j, i), dg


def _octa(od, fn, w, order, size, late=()):
    acc, ps = [[[], [], []] for _ in range(6)], {}
    todo = [n for n in range(48) if n not in late] + list(late)
    todo = [todo[k:k + size] for k in range(0, 48, size)]
    nodes = lambda n: order[n // 4] if n % 4 < 3 else order[n // 4][sum(order[n // 4]) % 2:][:1]

    def group(ns):
        for n in ns:
            i, j = order[n // 4]
            s, t = i // 2, j // 2
            e, x = (j, s) if (i + j) % 2 else (i, t)
            lhs = (lambda: fn(i, s) - fn(j, s), lambda: fn(j, t) - fn(i, t),
                   lambda: fn(i, t) - fn(j, s) if t == 2 else fn(i, t) + fn(j, s), lambda: fn(e, x))[n % 4]()
            ps[n] = _dot(od.group(lhs) if n == ns[0] else lhs, w(n))
            if n % 4 == 2:
                q = ps[n] + ps[n - 1] - ps[n - 2] if t == 2 else ps[n] + ps[n - 1] + ps[n - 2]
                acc[j][s].append(ps[n - 2])
                acc[i][t].append(ps[n - 1])
                acc[i][3 - s - t].append(q)
                acc[j][3 - s - t].append(q)
            elif n % 4 == 3:
                acc[e][x].append(ps[n] if n in late else acc[e][x].pop() + ps[n])
        od.issued(ps[n])

    def result(o, rows):
        assert all(n in ps for n in range(48) if o in nodes(n))
        a = [_total(a, rows) for a in acc[o]]
        return a[2] - a[1] if o < 2 else a[0], a[2] - a[0] if o // 2 == 1 else a[1]

    uses = [[g for g, ns in enumerate(todo) if any(c in nodes(n) for n in ns)] for c in range(6)]
    return [lambda ns=ns: group(ns) for ns in todo], result, uses


class _Order:
    def __init__(self, never):
        self.never, self.due, self.slot = never, {}, 0

    def run(self, task):
        self.task = task
        task.fn()
        self.slot += bool(task.time)

    def issued(self, p):
        self.last, self.row = p, 0

    def after(self, x):
        o = self.row % (self.last.shape[0] - PC + 8)
        self.row += PC
        head = jnp.where(jnp.concatenate([self.never] * (PC // 8), axis=0), self.last[o:o + PC, :128], x[:, :128])
        return head if x.shape[1] == 128 else jnp.concatenate([head, x[:, 128:]], axis=1)

    def soon(self, *xs):
        v = _total(xs, slice(None))
        self.due.setdefault(self.task.due, []).append(jnp.broadcast_to(v, (v.shape[0], 128)))

    def group(self, a, part=0, parts=1):
        vs = self.due.get(self.slot, [])
        vs = vs[len(vs) * part // parts:len(vs) * (part + 1) // parts]
        if not vs:
            return a
        v = jnp.concatenate(vs, axis=0)
        n, m = a.shape[0] // 8, v.shape[0] // 8
        k = max(d for d in range(1, m + 1) if n % d == 0)
        head = v[:m // k * k * 8].reshape(k, m // k, 8, 128).sum(axis=1)
        if m % k:
            head = jnp.concatenate([head[:-(m % k)], head[-(m % k):] + v[-(m % k) * 8:].reshape(-1, 8, 128)], axis=0)
        x = a[:, :128].reshape(k, n // k, 8, 128)
        last = jnp.where(self.never[None], lax.bitcast_convert_type(head, a.dtype), x[:, -1])[:, None]
        x = (jnp.concatenate([x[:, :-1], last], axis=1) if n > k else last).reshape(-1, 128)
        return x if a.shape[1] == 128 else jnp.concatenate([x, a[:, 128:]], axis=1)


class _Task:
    def __init__(self, fn, valu=0, store=0, time=0, needs=(), lag=0, spill=0):
        self.fn, self.valu, self.store, self.time, self.lag, self.spill = fn, valu, store, time, lag, spill
        self.needs, self.feeds = list(needs), []


def _schedule(main):
    fill = []

    def visit(task):
        for e in task.needs:
            e.feeds.append(task)
            if not e.time and len(e.feeds) == 1:
                visit(e)
                fill.append(e)
    for k, task in enumerate(main):
        task.slot, task.lo, task.hi, task.depth, task.height = k, k, k - 1, 0, 0
        visit(task)
    for e in fill:
        e.lo, e.depth = max([-1] + [p.lo for p in e.needs]), 1 + max([0] + [p.depth for p in e.needs])
    for e in reversed(fill):
        e.hi, e.height = min(n.hi for n in e.feeds), 1 + max(n.height for n in e.feeds)
        assert e.lo <= e.hi
    load = [[e.valu + p.spill, e.store + p.spill] for p, e in zip(main[-1:] + main, main)]
    cycles = lambda t, v, s: (t ** 4 + (v / 0.85) ** 4 + (s / 0.8) ** 4) ** 0.25

    def shares(e, slot):
        k = max(0, min([slot + 1 + e.lag, e.hi + 1] + [at for at, _ in WAITS if at >= slot]))
        early = (0.7 if e.lag else 0.3) * (k > 0)
        return (k - 1, early), (k, 1 - early)

    def put(e, sign):
        for k, part in shares(e, e.slot):
            load[k] = [load[k][0] + sign * part * e.valu, load[k][1] + sign * part * e.store]
        e.due = k

    def cost(e, slot):
        tight = sum(max(0, (1 if p.time else (slot < 110) * p.lag) - slot + p.slot) for p in e.needs)
        tight += sum(max(0, (1 + e.lag if n.time else (slot < 110) * e.lag) - n.slot + slot) for n in e.feeds)
        out = 10 * tight - 1e-4 * slot * e.lag
        for k, part in shares(e, slot):
            (v, s), t = load[k], main[k].time
            out += cycles(t, v + part * e.valu, s + part * e.store) - cycles(t, v, s)
        return round(out, 6)
    for e in fill:
        e.slot = max([e.lo + (e.hi - e.lo) * e.depth // (e.depth + e.height)] + [p.slot for p in e.needs])
        put(e, 1)
    for sweep in range(10):
        if sweep == 8:
            load[:] = [[v + 16 * (int(x) - 4), s + 16 * (int(x) - 4)] for (v, s), x in zip(load, BIAS)]
        for e in (fill if sweep % 2 else reversed(fill)):
            put(e, -1)
            first = max([-1] + [p.slot for p in e.needs])
            last = min(n.slot - bool(n.time) for n in e.feeds)
            e.slot = min(range(first, last + 1), key=lambda k: cost(e, k) + (sweep >= 8) * 0.03 * e.valu * abs(k - e.slot))
            put(e, 1)
    return sorted(main + fill, key=lambda e: (e.slot, not e.time))


def _merge(*jobs):
    keyed = [((k + 0.5) / len(job), n, e) for n, job in enumerate(jobs) for k, e in enumerate(job)]
    return [e for _, _, e in sorted(keyed, key=lambda e: e[:2])]


def _dft_matrices(mf, mi):
    sub, lane = (lax.broadcasted_iota(jnp.int32, (16, 128), d) for d in range(2))

    def turns(n):
        a = (n & (4 * T - 1)).astype(f32) * (-2 * np.pi / (4 * T))
        return jnp.cos(a), jnp.sin(a)
    mul = lambda a, b: (a[0] * b[0] - a[1] * b[1], a[0] * b[1] + a[1] * b[0])
    m, n = 4 * (sub & 7) + 1, 4 * ((lane >> 4) * 8 + (lane & 7)) + 1
    fwd, fwd_p = turns(m * R * lane + T * (sub >> 3)), tuple(jnp.concatenate([x, x], axis=0) for x in turns(m[:8]))
    fwd_a, fwd_ap = turns(32 * R * lane[:1]), (np.cos(16 * np.pi / T), -np.sin(16 * np.pi / T))
    inv, inv_p, inv_a = turns(n * R * sub + T * ((lane >> 3) & 1)), turns(n[:1]), turns(16 * R * n[:1])
    inv_h, inv_hp = ((1 - 2 * (sub & 1)).astype(f32), 0.0), (np.sqrt(0.5), -np.sqrt(0.5))
    for p in range(R):
        x = fwd
        for a in range(0, 256, 16):
            mf[p, a:a + 16] = x[0].astype(bf16)
            x = mul(x, fwd_a)
        for hf, x in enumerate((inv, mul(inv, inv_h))):
            for a in range(128 * hf, 128 * hf + 128, 16):
                mi[p, a:a + 16] = x[0].astype(bf16)
                x = mul(x, inv_a)
        fwd, fwd_a, inv, inv_h = mul(fwd, fwd_p), mul(fwd_a, fwd_ap), mul(inv, inv_p), mul(inv_h, inv_hp)


def _kernel(q_hbm, k_hbm, v_hbm, sk_hbm, g_hbm, sd_hbm, w1_hbm, w2_hbm, w3_hbm, w4_hbm, o_hbm,
            sk, sd, qb, kb, vb, gb, w1, w2, w3, w4, c1, c2, c3, c4, mf, mi, wz, gt, yb, xb, xn, xo, n3, hb, ob,
            sem_i, sem_o):
    tile = lambda x, c: x[:, c * 128:(c + 1) * 128]
    cols = lambda c: pl.ds(c * 128, 128)
    flat = lambda ps: [e for p in ps for e in p]

    def conv_in(j, c):
        rows, lead = pl.ds(j * T, T), 16 * (j > 0)
        block = cols(c) if isinstance(c, int) else pl.ds(pl.multiple_of(c * 128, 128), 128)
        return [(k_hbm.at[pl.ds(j * T - lead, T + lead), block], kb.at[j, c, pl.ds(16 - lead, T + lead), :]),
                (v_hbm.at[rows, block], vb.at[j, c, pl.ds(0, T), :]),
                (g_hbm.at[block, rows], gb.at[j, c])]

    def wait(n, keys):
        each = lambda pairs: [pltpu.make_async_copy(src, dst, sem_i.at[n]).wait() for src, dst in pairs]
        for key in keys:
            if key in (2, 3):
                @pl.loop(0, NB)
                def _(c):
                    each(conv_in(key, c))
            else:
                each(inputs[key])

    inputs = {(j, c): conv_in(j, c) for j in range(2) for c in range(NB)}
    inputs[0, 0] += [(sk_hbm, sk), (sd_hbm, sd)]
    inputs.update({j: flat(conv_in(j, c) for c in range(NB)) for j in (2, 3)})
    inputs.update({'q%d' % j: [(q_hbm.at[pl.ds(j * T, T), :], qb.at[j])] for j in range(NT)})
    inputs.update({'w3' + 'ab'[e]: [(w3_hbm.at[:, pl.ds(e * F // 2, F // 2)], w3.at[e])] for e in range(2)})
    inputs.update({'w1': [(w1_hbm, w1)], 'w2': [(w2_hbm, w2)], 'w4': [(w4_hbm, w4)]})
    got, sent = {}, []
    for n, (_, keys) in enumerate(WAITS):
        for src, dst in flat(inputs[key] for key in keys):
            pltpu.make_async_copy(src, dst, sem_i.at[n]).start()
        got.update(dict.fromkeys(keys, _Task(lambda n=n, keys=keys: wait(n, keys))))

    for c in range(NB):
        kb[0, c, pl.ds(0, 16), :] = jnp.zeros((16, 128), bf16)
        for l in range(2):
            hb[l, c, pl.ds(0, HP), :] = jnp.zeros((HP, 128), f32)
            hb[l, c, pl.ds(HP + S, HP), :] = jnp.zeros((HP, 128), f32)
    _dft_matrices(mf, mi)
    mf, mi = mf.bitcast(u32), mi.bitcast(u32)
    od = _Order(mf[0, 0:8, :] == np.uint32(0xFFFFFFFF))
    kw, vw = kb.bitcast(u32), vb.bitcast(u32)

    spec = {}

    def conv(j, c, prev):
        def put(o, xs):
            for p, x in enumerate(xs):
                wz[c, p, pl.ds(o, 16), :] = x.astype(bf16)

        def pre_t():
            gt[c, pl.ds(0, T // 2), :] = pltpu.bitcast(gb[j, c].T, u32)

        def pre_u(o):
            s = tile(sk[...], c).astype(f32) * (1.0 / T)
            s0, s1, s2, s3 = (s[i:i + 1] for i in range(4))
            ld = lambda ref, w: ref[j, c, pl.ds(2 * o + w, 16, stride=2), :]
            wa, wb, pa, pb, va, vc = ld(kw, 8), ld(kw, 9), ld(kw, 6), ld(kw, 7), ld(vw, 0), ld(vw, 1)
            k0, k1, k2, k3, m1, m2, m3 = _lo(wa), _hi(wa), _lo(wb), _hi(wb), _hi(pb), _lo(pb), _hi(pa)
            xs = [
                (s0 * k0 + s1 * m1 + s2 * m2 + s3 * m3) * _lo(va),
                (s0 * k1 + s1 * k0 + s2 * m1 + s3 * m2) * _hi(va),
                (s0 * k2 + s1 * k1 + s2 * k0 + s3 * m1) * _lo(vc),
                (s0 * k3 + s1 * k2 + s2 * k1 + s3 * k0) * _hi(vc)]
            put(o, xs)
            od.soon(jnp.concatenate(xs, axis=0))

        def pre_g(o):
            ga, gc = (gt[c, pl.ds(2 * o + w, 16, stride=2), :] for w in range(2))
            xs = _lo(ga), _hi(ga), _lo(gc), _hi(gc)
            put(128 + o, xs)
            od.soon(xs[0], xs[2])

        def spectrum(o):
            a = [_dot(_unpack(mf[p] if p else od.group(mf[p])), _unpack(wz.bitcast(u32)[c, p, o:o + 64])) for p in range(R)]
            od.issued(a[0])
            a = [(x[:, :8].reshape(128, 128), x[:, 8:].reshape(128, 128)) for x in (x.reshape(16, 16, 128) for x in a)]
            if o and j == 0:
                a[0] = (a[0][0] + sd[...].astype(f32)[c:c + 1], a[0][1])
            a = _bfly(a, False)
            for n in range(1, j + 1) if o else ():
                a = [(xr - yi, xi + yr) if n == 1 else (xr + yr, xi + yi) if n == 2 else (xr + yi, xi - yr)
                     for (xr, xi), (yr, yi) in zip(a, spec[c, j - n, o])]
            spec[c, j, o] = a

        def pre_y(o):
            zs = []
            for q in range(R):
                zr = zi = None
                for n in range(j + 1):
                    (gr, gi), (ur, ui) = ([x[8 * o:8 * o + 8] for x in spec[key][q]] for key in ((c, n, 64), (c, j - n, 0)))
                    zr, zi = _axpy(zr, 1, gr * ur - gi * ui), _axpy(zi, 1, gr * ui + gi * ur)
                zs.append((zr, zi))
            xs = [jnp.concatenate(b, axis=0) for b in _bfly(zs, True)]
            put(256 + 16 * o, xs)
            od.soon(xs[1])

        def inverse():
            for p in range(R):
                m = mi[p, :64] if p % 2 else od.group(mi[p, :64], p // 2, 2)
                y = _dot(jnp.concatenate([_unpack(m), _unpack(mi[p, 64:])], axis=1), _unpack(wz.bitcast(u32)[c, p, 128:]))
                yb[c, pl.ds(j * T + p, 128, stride=R), :] = y
            od.issued(y)

        ahead = lambda needs: [_Task(lambda: None, needs=needs, lag=1)]
        free = [got[(j, c) if j < 2 else j]] + prev
        tr = _Task(pre_t, 8, 32, needs=free)
        u = _Task(lambda: spectrum(0), 100, 128, 256, spill=80, needs=ahead(
            [_Task(lambda o=o: pre_u(o), 24, 8, needs=free) for o in range(0, 128, 16)]))
        g = _Task(lambda: spectrum(64), 140, 128, 256, spill=80 + 16 * j, needs=ahead(
            [_Task(lambda o=o: pre_g(o), 4, 4, needs=[tr]) for o in range(0, 128, 16)]))
        y = _Task(inverse, 32, 64, 256, needs=ahead(
            [_Task(lambda o=o: pre_y(o), 8 * j + 10, 8, needs=[u, g]) for o in range(16)]))
        return u, g, y

    def slab(w, i, j, o):
        return w[pl.ds(i * 128 + o, 16), cols(j)].astype(f32)

    def keep(cw, first, step, o, xs):
        for k, x in enumerate(xs):
            cw[first + step * k, pl.ds(o, 16), :] = x.astype(bf16)
        od.soon(jnp.concatenate(xs[3::4], axis=0))

    def prep_star(block, cw, needs):
        def piece(o):
            b = [[block(i, j, o) for j in range(NB)] for i in range(NB)]
            keep(cw, 0, 1, o, flat(_star_weights(b, g) for g in range(len(STAR))))
        return [_Task(lambda o=o: piece(o), 70, 60, needs=needs) for o in range(0, 128, 16)]

    def prep_octa(block, cw, order, swap, needs):
        def piece(e, o):
            b = {}
            for n in range(6):
                x = [block(k, n, e, o) for k in range(NB)]
                for k in range(6):
                    if k != n ^ 1:
                        b[(n, k) if swap else (k, n)] = x[k] if n == 4 else x[n ^ 1] if k == 5 else x[k] - x[n ^ 1]
            keep(cw, e, 2, o, flat(_octa_weights(lambda i, j: b[i, j], i, j) for i, j in order))
        return [_Task(lambda e=e, o=o: piece(e, o), 85, 80, needs=[needs[e]]) for e in range(2) for o in range(0, 128, 16)]

    def rstd(st, scale, needs):
        def piece():
            st[1] = _rstd(*st, scale)
            od.soon(st[1])
        return _Task(piece, 11, 6, needs=needs, lag=1)

    inner = {}

    def gate(r, needs):
        st, rows = [], pl.ds(r % S, PC)

        def piece(stage):
            x = xb[rows, :] if stage == 2 else qb[r // T, pl.ds(r % T, PC), :].astype(f32) if r < S else xo[rows, :]
            if stage == 0:
                x = od.after(x)
            elif stage == 1:
                x = x + _norm(x, od.after(st[0]), st[1]) * jnp.concatenate([yb[c, rows, :] for c in range(NB)], axis=1)
                xb[rows, :] = x
            else:
                x = _norm(x, od.after(st[0]), st[1])
                xn[rows, :] = x
            st[:] = _sums(x)
            od.soon(st[1][-8:])
        task = []
        for stage, (valu, store) in enumerate(((20, 10), (42, 35), (30, 35))):
            task = [_Task(lambda stage=stage: piece(stage), valu, store, lag=1,
                          needs=(task and [rstd(st, 1, task)]) + (needs[0], needs[1], [])[stage])]
        inner[r] = st, rstd(st, GS, task)
        return task[0]

    def square(src, w, cw, scale, h, fast, needs):
        if fast:
            groups, result = _star(od, src, lambda k: _unpack(cw.bitcast(u32)[k]))
            groups = [_Task(fn, 0.26 * h, 0.4 * h, h) for fn in groups]
            last = [[x for x, e in zip(groups, STAR) if c in e][-1:] for c in range(NB)]
        else:
            f, out = {}, {}

            def group(g):
                for n in range(g, min(g + 4, NB * NB)):
                    c, k = divmod(n, NB)
                    if k not in f:
                        f[k] = jnp.concatenate(src(k), axis=0)
                    out[c] = _axpy(out.get(c), 1, _dot(od.group(f[k]) if n == g else f[k], w[cols(k), cols(c)]))
                od.issued(out[c])
            groups = [_Task(lambda g=g: group(4 * g), 0.1 * h * n, 0.1 * h * n, h * n / 2)
                      for g, n in enumerate((4,) * 6 + (1,))]
            result = lambda c, rows: [_axpy(None, scale, out[c][hf * h:][rows]) for hf in range(2)]
            last = [[groups[(NB * c + NB - 1) // 4]] for c in range(NB)]
        groups[0].needs += needs
        return groups, result, last

    def mm1(r0, h, fast, needs):
        src = lambda c: [xn[pl.ds(r0 % S + hf * h, h), cols(c)] for hf in range(2)]
        groups, result, last = square(src, w1, c1, 1, h, fast, needs)

        def post(c, o):
            xs = [_gelu((x if fast else x - s * tile(col_mean[0], c)) * r) for x, (s, r) in zip(
                result(c, slice(o, o + PC)), (inner[r0 + hf * h + o][0] for hf in range(2)))]
            for hf in range(2):
                hb[r0 // S, c, pl.ds(r0 % S + HP + hf * h + o, PC), :] = xs[hf]
            od.soon(*xs)
        return groups, [_Task(lambda c=c, o=o: post(c, o), 27, 14,
                              needs=last[c] + [mean1, inner[r0 + o][1], inner[r0 + h + o][1]])
                        for c in range(NB) for o in range(0, h, PC)]

    def mm2(r0, h, to, fast, needs):
        def shifted(c, r):
            ld = lambda sh: hb[r // S, c, pl.ds(r % S + HP - sh, h), :]
            sh, lane = (1, -1, 2, -2), lax.broadcasted_iota(jnp.int32, (h, 128), 1)
            return ld(sh[0]) if c == 0 else ld(sh[3]) if c == 4 else jnp.where(lane < 32 * c, ld(sh[c - 1]), ld(sh[c]))
        groups, result, last = square(lambda c: (shifted(c, r0), shifted(c, r0 + h)), w2, c2, GO, h, fast, needs)

        def post(c, o):
            for hf, x in enumerate(result(c, slice(o, o + PC))):
                xn[pl.ds(r0 % S + hf * h + o, PC), cols(c)] += x

        def sums(o, st):
            st[:] = _sums(od.after(xn[pl.ds(r0 % S + o, PC), :]))
            od.soon(st[1][-8:])

        def norm(o, st):
            n = _norm(xn[pl.ds(r0 % S + o, PC), :], od.after(st[0]), st[1])
            v = _total([tile(n, c) for c in range(NB)], slice(None))
            n3[pl.ds(to + o, PC), :] = jnp.concatenate([n, v], axis=1)
            od.soon(v)
        out = []
        for o in range(0, h, PC):
            posts = [_Task(lambda c=c, o=o: post(c, o), needs=last[c]) for c in range(NB)]
            for p, st in ((o, []), (h + o, [])):
                task = _Task(lambda p=p, st=st: sums(p, st), 48, 27, needs=posts, lag=1)
                out.append(_Task(lambda p=p, st=st: norm(p, st), 20, 30, needs=[rstd(st, GS, [task])], lag=1))
        return groups, out

    def mm34(r0, h, needs3, needs4):
        act, common = {}, {}

        def src(c, x):
            a, b = n3[pl.ds(0, h), cols(c)], n3[pl.ds(h, h), cols(c)]
            return a + b if x == 2 else (a, b)[x]
        m3 = [_octa(od, src, lambda k, e=e: _unpack(c3.bitcast(u32)[2 * k + e]), ORD3, 4) for e in range(2)]
        g4, result4, uses4 = _octa(od, lambda c, x: jnp.concatenate(
            [jnp.concatenate([act[n, o][x] for o in range(0, h, PC)], axis=0) for n in PAIR4[c]], axis=1),
            lambda k: jnp.concatenate([_unpack(c4.bitcast(u32)[2 * k]), _unpack(c4.bitcast(u32)[2 * k + 1])], axis=0), ORD4, 2,
            late=(31, 47, 35, 39) * (r0 + 2 * h == 2 * S))
        g3 = [_Task(fn, 0.26 * h, 0.39 * h, h) for fn in m3[0][0] + m3[1][0]]
        g4 = [_Task(fn, 0.31 * h, 0.25 * h, h) for fn in g4]

        def post3(n, o):
            a, b = (_gelu(x) for x in m3[n // 6][1](n % 6, slice(o, o + PC)))
            act[n, o] = a, b, a + b
            od.soon(act[n, o][2])

        def post4(c, o):
            xs = result4(c, slice(o, o + PC))
            if c == 5:
                common[o] = xs
                return
            for hf in range(2):
                rows = pl.ds(r0 % S + hf * h + o, PC)
                x = xb[rows, cols(c)] + xn[rows, cols(c)] + common[o][hf] + xs[hf]
                if r0 < S:
                    xo[rows, cols(c)] = x
                else:
                    ob[c, rows, :] = x.astype(bf16)

        def send(c):
            rows = pl.ds(r0 - S, 2 * h)
            sent.append(pltpu.make_async_copy(ob.at[c, rows, :], o_hbm.at[rows, cols(c)], sem_o.at[0]))
            sent[-1].start()
        g3[0].needs += needs3[0]
        g3[12].needs += needs3[1]
        g4[0].needs += needs4
        for c in range(6):
            g4[uses4[c][0]].needs += [
                _Task(lambda n=n, o=o: post3(n, o), 24, 18, needs=[g3[n // 6 * 12 + m3[0][2][n % 6][-1]]])
                for n in PAIR4[c] for o in range(0, h, PC)]
        p4 = {}
        for c in (5, 0, 1, 2, 3, 4):
            p4[c] = [_Task(lambda c=c, o=o: post4(c, o), 8, 4,
                           needs=[g4[uses4[c][-1]]] + ([p4[5][o // PC]] if c < 5 else []))
                     for o in range(0, h, PC)]
        return g3, g4, flat(p4[c] if r0 < S else [_Task(lambda c=c: send(c), needs=p4[c])] for c in range(NB))

    parts, col_mean = [], []
    for j in range(NT):
        parts.append([conv(j, c, [parts[-1][c][2]] if j else []) for c in range(NB)])
    cv = [[parts[j][int(e[1])]['ugy'.index(e[0])] for e in CONV[j].split()] for j in range(NT)]
    mean1 = _Task(lambda: col_mean.append(jnp.sum(w1[...].astype(f32), axis=0, keepdims=True) * (1.0 / D)),
                  200, 10, needs=[got['w1']])
    pr1 = prep_star(lambda i, j, o: slab(w1, i, j, o) - tile(col_mean[0], j), c1, [mean1])
    pr2 = prep_star(lambda i, j, o: slab(w2, i, j, o) * GO, c2, [got['w2']])
    pr3 = prep_octa(lambda k, n, e, o: slab(w3.at[e], k, n, o), c3, ORD3, False, [got['w3a'], got['w3b']])
    pr4 = prep_octa(lambda k, n, e, o: slab(w4, PAIR4[n][e], k, o) * GO, c4, ORD4, True, [got['w4']] * 2)
    edges = [[0] + [i * T - k * OFF for i in range(1, NT)] + [S] for k in range(3)]
    g1, g2, g3, g4, done = [], [], [], [], []
    for t, (l, i) in enumerate(TILES):
        (a0, a1), (b0, b1) = edges[l][i:i + 2], edges[l + 1][i:i + 2]
        if l:
            needs = [cv[1][0] if t == 1 else g3[t - 1][0]], []
        else:
            needs = [got['q%d' % i]] + (g1[t - 2][-1:] if t > 1 else []), [p[2] for p in parts[i]]
        pre = [gate(l * S + r, needs) for r in range(a0, a1, PC)]
        if t < 2:
            n = a1 - T // 2
            (a, pa), (b, pb) = (mm1(l * S + r, m // 2, False, pre[r // PC:(r + m) // PC] + [got['w1']])
                                for r, m in ((0, n), (n, a1 - n)))
            a += b
        else:
            (a, pa), pb = mm1(l * S + a0, (a1 - a0) // 2, True, pre + (pr1 if t == 2 else [])), []
        if t == 0:
            n -= OFF
            (c, pc), (d, pd) = mm2(0, n // 2, 0, False, pa + [got['w2']]), mm2(n, (b1 - n) // 2, n, False, pb)
            c, pc = c + d, pc + pd
        else:
            c, pc = mm2(l * S + b0, (b1 - b0) // 2, 0, True, pa + pb + (pr2 if t == 1 else []))
        x3, x4, fin = mm34(l * S + b0, (b1 - b0) // 2, (pc, []) if t else (pc + pr3[:8], pr3[8:]), [] if t else pr4)
        for lst, e in zip((g1, g2, g3, g4), (a, c, x3, x4)):
            lst.append(e)
        (cv[1][0] if t == 1 else x3[0]).needs += done
        done = fin

    main = cv[0] + g1[0] + g2[0] + g3[0] + g4[0] + cv[1][:4] + g1[1] + cv[1][4:5] + _merge(g2[1], cv[1][5:6]) + cv[1][6:9]
    for t, (a, b) in enumerate(CUTS, 1):
        main += g3[t] + g4[t][:a] + g1[t + 1] + g4[t][a:b] + g2[t + 1] + g4[t][b:]
    main += g3[-1] + g4[-1] + [_Task(lambda: [cp.wait() for cp in sent], time=1, needs=done)]
    for j, first, lo, hi in SPANS:
        main[lo:hi] = _merge(main[lo:hi], cv[j][first:])
    for at, keys in WAITS:
        got[keys[0]].needs += main[at:at + 1]
        main[at + 1].needs.append(got[keys[0]])
    for task in _schedule(main):
        od.run(task)


@jax.jit
def pallas_interleave_layers__ssm_conv_h3__mixer_s_mlp__prompt_kernel(
        A_q, A_k, A_v, A_shift_k, A_ssm_k, A_ssm_D, B_x, B_w1, B_w2, B_w3, B_w4):
    del B_x
    hbm, vmem = pl.BlockSpec(memory_space=pl.ANY), pltpu.VMEM
    out = pl.pallas_call(
        _kernel,
        out_shape=jax.ShapeDtypeStruct((S, D), bf16),
        in_specs=[hbm] * 10,
        out_specs=hbm,
        scratch_shapes=[
            vmem((4, D), bf16), vmem((NB, 128), bf16), vmem((NT, T, D), bf16),
            vmem((NT, NB, T + 32, 128), bf16), vmem((NT, NB, T + 16, 128), bf16),
            vmem((NT, NB, 128, T), bf16),
            vmem((D, D), bf16), vmem((D, D), bf16), vmem((2, D, F // 2), bf16), vmem((F, D), bf16),
            vmem((40, 128, 128), bf16), vmem((40, 128, 128), bf16),
            vmem((96, 128, 128), bf16), vmem((96, 128, 128), bf16),
            vmem((R, 256, 128), bf16), vmem((R, 256, 128), bf16),
            vmem((NB, R, 512, 128), bf16), vmem((NB, T // 2 + 8, 128), u32),
            vmem((NB, S + 8, 128), f32),
            vmem((S, D), f32), vmem((S, D), f32), vmem((S, D), f32),
            vmem((T + 2 * OFF, D + 128), f32),
            vmem((2, NB, S + 2 * HP, 128), f32), vmem((NB, S, 128), bf16),
            pltpu.SemaphoreType.DMA((len(WAITS),)), pltpu.SemaphoreType.DMA((1,)),
        ],
        compiler_params=pltpu.CompilerParams(vmem_limit_bytes=120 * 1024 * 1024),
    )(A_q.reshape(S, D), A_k.reshape(S, D), A_v.reshape(S, D), A_shift_k.T, A_ssm_k, A_ssm_D.reshape(NB, 128),
      B_w1, B_w2, B_w3, B_w4)
    return out.reshape(1, S, D)
```
